```python
import jax
import jax.numpy as jnp

def _softmax(x, axis=-1):
    return jax.nn.softmax(x, axis=axis)
def _gelu(x):
    return jax.nn.gelu(x, approximate=True)
def _silu(x):
    return jax.nn.silu(x)
def _sigmoid(x):
    return jax.nn.sigmoid(x)
def _layernorm(x, axis=-1, eps=1e-5):
    m = jnp.mean(x, axis=axis, keepdims=True)
    v = jnp.var(x, axis=axis, keepdims=True)
    return (x - m) / jnp.sqrt(v + eps)
def _scatter_add(tgt, idx, src, axis=0):
    return tgt.at[idx].add(src)
def _segment_sum(src, seg, n):
    return jax.ops.segment_sum(src, seg, n)
class _Rng:
    def __init__(self, key):
        self._k = key
    def _next(self):
        self._k, sub = jax.random.split(self._k)
        return sub
    def normal(self, shape):
        return jax.random.normal(self._next(), shape, dtype=jnp.bfloat16)
    def randint(self, lo, hi, shape):
        return jax.random.randint(self._next(), shape, lo, hi, dtype=jnp.int32)
    def uniform(self, shape, lo=0.0, hi=1.0):
        return jax.random.uniform(self._next(), shape, jnp.bfloat16, lo, hi)
    def permutation(self, n):
        return jax.random.permutation(self._next(), n)


kernel_name = 'sequential_preLN__compressed_kv_cla__moe_arch_mod__prompt'

def setup_inputs():
    _rng = _Rng(jax.random.key(int.from_bytes(__import__("os").urandom(4), "little")))
    _w = (lambda a: (lambda t: t.astype(jnp.bfloat16) if jnp.issubdtype(t.dtype, jnp.floating) else t)(jnp.asarray(a)))
    def _A_setup():
        B, H, Sq, Sk, D, M = 1, 32, 2048, 2048, 128, 1024
        Dc = 4 * D
        return {
            "x": _w((lambda *s: _rng.normal(s) * 0.05)(B, Sq, M)),
            "c_kv": _w((lambda *s: _rng.normal(s) * 0.05)(B, Sk, Dc)),
            "w_q": _w((lambda *s: _rng.normal(s) * 0.05)(M, H, D) * (M ** -0.5)),
            "w_uk": _w((lambda *s: _rng.normal(s) * 0.05)(Dc, H, D) * (Dc ** -0.5)),
            "w_uv": _w((lambda *s: _rng.normal(s) * 0.05)(Dc, H, D) * (Dc ** -0.5)),
            "w_o": _w((lambda *s: _rng.normal(s) * 0.05)(H, D, M) * ((H * D) ** -0.5)),
        }
    _A_in = _A_setup()

    def _B_setup():
        B, S, D, F, C = 1, 2048, 1024, 3584, 2
        return {
            "x": _w((lambda *s: _rng.normal(s) * 0.05)(B, S, D)),
            "w_r": _w((lambda *s: _rng.normal(s) * 0.05)(D)),
            "w_gate": _w((lambda *s: _rng.normal(s) * 0.05)(D, F)),
            "w_up": _w((lambda *s: _rng.normal(s) * 0.05)(D, F)),
            "w_down": _w((lambda *s: _rng.normal(s) * 0.05)(F, D)),
        }
    _B_in = _B_setup()

    return {
        "A_x": _A_in["x"],
        "A_c_kv": _A_in["c_kv"],
        "A_w_q": _A_in["w_q"],
        "A_w_uk": _A_in["w_uk"],
        "A_w_uv": _A_in["w_uv"],
        "A_w_o": _A_in["w_o"],
        "B_x": _B_in["x"],
        "B_w_r": _B_in["w_r"],
        "B_w_gate": _B_in["w_gate"],
        "B_w_up": _B_in["w_up"],
        "B_w_down": _B_in["w_down"],
    }

def reference(A_x, A_c_kv, A_w_q, A_w_uk, A_w_uv, A_w_o, B_x, B_w_r, B_w_gate, B_w_up, B_w_down):
    def _A_ref(x, c_kv, w_q, w_uk, w_uv, w_o):
        B, Sq, M = x.shape[0], x.shape[1], x.shape[2]
        Sk = c_kv.shape[1]
        H, D = w_q.shape[1], w_q.shape[2]
        q = jnp.einsum("bqm,mhd->bhqd", x, w_q)
        k = jnp.einsum("bkc,chd->bhkd", c_kv, w_uk)
        v = jnp.einsum("bkc,chd->bhkd", c_kv, w_uv)
        scores = jnp.einsum("bhqd,bhkd->bhqk", q, k) * (D ** -0.5)
        off = Sk - Sq
        qi = jnp.arange(Sq)[:, None]
        kj = jnp.arange(Sk)[None, :]
        cmask = kj <= (qi + off)
        scores = jnp.where(cmask[None, None], scores, -1e9)
        p = _softmax(scores, axis=-1)
        ctx = jnp.einsum("bhqk,bhkd->bhqd", p, v)
        return jnp.einsum("bhqd,hdm->bqm", ctx, w_o)

    def _B_ref(x, w_r, w_gate, w_up, w_down):
        B, S, D = x.shape
        C = 2
        r = x @ w_r
        idx = jnp.argsort(-r, axis=-1)[:, :C]
        idx_e = jnp.repeat(idx.reshape(B, C, 1), D, axis=2)
        x_sel = jnp.take_along_axis(x, idx_e, axis=1)
        g = _silu(x_sel @ w_gate)
        u = x_sel @ w_up
        y = (g * u) @ w_down
        r_sel = _sigmoid(jnp.take_along_axis(r, idx, axis=1))
        y = y * r_sel.reshape(B, C, 1)
        b_off = (jnp.arange(B) * S).reshape(B, 1)
        flat_idx = (idx + b_off).reshape(B * C)
        zero = (x * 0.0).reshape(B * S, D)
        upd = _scatter_add(zero, flat_idx, y.reshape(B * C, D), axis=0)
        return x + upd.reshape(B, S, D)

    x = A_x
    h = x + _A_ref(_layernorm(x, axis=-1), A_c_kv, A_w_q, A_w_uk, A_w_uv, A_w_o)
    h2 = h + _B_ref(_layernorm(h, axis=-1), B_w_r, B_w_gate, B_w_up, B_w_down)
    return h2
```

```python
import functools
import jax, jax.numpy as jnp
from jax import lax
from jax.experimental import pallas as pl
from jax.experimental.pallas import tpu as pltpu

S, M, H, D, DC, F = 2048, 1024, 32, 128, 512, 3584
BQ = 512
T = 128
RC = 256
LG = 32
PC = 512
PLACE = (0,0,3,3,6,6,10,15)
f32, bf16, u32, i32 = jnp.float32, jnp.bfloat16, jnp.uint32, jnp.int32
QSC = (D ** -0.5) * 1.4426950408889634
NEG = -1e30
EPS = 1e-5


def _dot(a, b):
    return jnp.dot(a, b, preferred_element_type=f32)


def _dot_nt(a, b):
    return lax.dot_general(a, b, (((1,), (1,)), ((), ())), preferred_element_type=f32)


def _rb(x):
    return x.astype(bf16).astype(f32)


def _cat(xs, axis):
    return xs[0] if len(xs) == 1 else jnp.concatenate(xs, axis=axis)


def _tiles(x):
    return [x[:, j * T:(j + 1) * T] for j in range(x.shape[1] // T)]


def _attend_steps(q_ref, k_ref, v_ref, o_ref, bias):
    nt = BQ // T

    def qk(I):
        r0 = I * BQ
        q = q_ref[r0:r0 + BQ, :]
        sr = _tiles(_dot_nt(q, k_ref[:r0, :])) if I else []
        sd = [_dot_nt(q[t * T:], k_ref[r0 + t * T:r0 + (t + 1) * T, :]) for t in range(nt)]
        return sr, sd

    def softmax(s):
        sr, sd = s
        n = len(sr)
        pd = [[] for _ in range(nt)]
        pr, ls = [], []
        for r in range(nt):
            pcs = [x[r * T:(r + 1) * T] for x in sr] + [sd[t][(r - t) * T:(r - t + 1) * T] for t in range(r + 1)]
            pcs[-1] = pcs[-1] + bias
            m = jnp.max(functools.reduce(jnp.maximum, pcs), axis=1, keepdims=True)
            ps = [jnp.exp2(x - m).astype(bf16) for x in pcs]
            ls.append(jnp.sum(functools.reduce(jnp.add, [x.astype(f32) for x in ps]), axis=1, keepdims=True))
            if n:
                pr.append(_cat(ps[:n], 1))
            for t in range(r + 1):
                pd[t].append(ps[n + t])
        return pr, pd, ls

    def pv(I, p):
        pr, pd, ls = p
        r0 = I * BQ
        orr = _dot(_cat(pr, 0), v_ref[:r0, :]) if I else None
        os_ = [_dot(_cat(pd[t], 0), v_ref[r0 + t * T:r0 + (t + 1) * T, :]) for t in range(nt)]
        for r in range(nt):
            pcs = [os_[t][(r - t) * T:(r - t + 1) * T] for t in range(r + 1)]
            if I:
                pcs.append(orr[r * T:(r + 1) * T])
            l = ls[r]
            inv = pl.reciprocal(l, approx=True)
            inv = inv * (2.0 - l * inv)
            o_ref[r0 + r * T:r0 + (r + 1) * T, :] = (functools.reduce(jnp.add, pcs) * inv).astype(bf16)

    order = list(range(S // BQ))[::-1]
    st = {}
    steps = [lambda: st.__setitem__(0, qk(order[0]))]
    for n, I in enumerate(order):
        if n + 1 < len(order):
            steps.append(lambda n=n: st.__setitem__(n + 1, qk(order[n + 1])))
        steps.append(lambda n=n, I=I: pv(I, softmax(st.pop(n))))
    return steps


def _kernel(x_hbm, c_hbm, wq_hbm, wk_hbm, wv_hbm, wo_hbm, wr_ref, wg_hbm, wu_hbm, wd_hbm, out_hbm,
            x_v, xn_v, c_v, wq_r, wk_r, wv_r, q_v, k_v, v_v, ctx_v, wo_v, wg_v, wu_v, wd_v, out_v, a_v,
            sems, csems, osems):
    wq32, wk32, wv32 = wq_hbm.bitcast(u32), wk_hbm.bitcast(u32), wv_hbm.bitcast(u32)

    def wcopies(p, s):
        return (pltpu.make_async_copy(wq32.at[:, p, :], wq_r.at[s], sems.at[s]),
                pltpu.make_async_copy(wk32.at[:, p, :], wk_r.at[s], sems.at[2 + s]),
                pltpu.make_async_copy(wv32.at[:, p, :], wv_r.at[s], sems.at[4 + s]))
    cp_c = [pltpu.make_async_copy(c_hbm.at[:, j * T:(j + 1) * T], c_v.at[j], csems.at[j]) for j in range(DC // T)]
    cp_x = [pltpu.make_async_copy(x_hbm.at[i * PC:(i + 1) * PC], x_v.at[i * PC:(i + 1) * PC], osems.at[i]) for i in range(S // PC)]
    big = [[pltpu.make_async_copy(a.at[:, j * T:(j + 1) * T], b.at[j], sems.at[8 + i]) for j in range(b.shape[0])]
           for i, (a, b) in enumerate([(wo_hbm, wo_v), (wg_hbm, wg_v), (wu_hbm, wu_v), (wd_hbm, wd_v)])]

    cq, ck, cv = wcopies(0, 0)
    ck.start(); cv.start()
    for cp in cp_c:
        cp.start()
    cq.start()
    for cp in cp_x:
        cp.start()

    def unpack(ref, h):
        w = ref[(h // 2) % 2]
        w = (w << ((1 - h % 2) * 16).astype(u32)) & jnp.uint32(0xFFFF0000)
        return pltpu.bitcast(w, f32).astype(bf16)

    def proj_steps(h, which="qkv"):
        s = h % 2
        w = {}
        steps = []
        for name, raw, src, n, dst, sc in (("k", wk_r, c_v, DC // T, k_v, None), ("v", wv_r, c_v, DC // T, v_v, None),
                                           ("q", wq_r, xn_v, M // T, q_v, QSC)):
            if name not in which:
                continue
            steps.append(lambda name=name, raw=raw: w.__setitem__(name, unpack(raw, h)))
            for i in range(S // PC):
                def f(name=name, src=src, n=n, dst=dst, sc=sc, i=i):
                    rows = slice(i * PC, (i + 1) * PC)
                    r = _dot(_cat([src[j, rows, :] for j in range(n)], 1), w[name])
                    if sc is not None:
                        r = r * sc
                    dst[s, rows, :] = r.astype(bf16)
                steps.append(f)
        return steps

    for cp in cp_c:
        cp.wait()
    ck.wait(); cv.wait()
    for f in proj_steps(jnp.int32(0), "kv"):
        f()
    cq.wait()
    wq0 = unpack(wq_r, jnp.int32(0))
    for i in range(S // PC):
        cp_x[i].wait()
        for g in range(PC // LG):
            rows = slice(i * PC + g * LG, i * PC + (g + 1) * LG)
            x = x_v[rows, :].astype(f32)
            xc = x - jnp.mean(x, axis=-1, keepdims=True)
            xn = (xc * lax.rsqrt(jnp.mean(xc * xc, axis=-1, keepdims=True) + EPS)).astype(bf16)
            for j in range(M // T):
                xn_v[j, rows, :] = xn[:, j * T:(j + 1) * T]
        rows = slice(i * PC, (i + 1) * PC)
        q_v[0, rows, :] = (_dot(_cat([xn_v[j, rows, :] for j in range(M // T)], 1), wq0) * QSC).astype(bf16)

    row = lax.broadcasted_iota(i32, (T, T), 0)
    col = lax.broadcasted_iota(i32, (T, T), 1)
    bias = jnp.where(col <= row, 0.0, NEG).astype(f32)

    def att_steps(h):
        s = h % 2
        return _attend_steps(q_v.at[s], k_v.at[s], v_v.at[s], ctx_v.at[h], bias)

    def body(h, _):
        @pl.when(h % 2 == 1)
        def _():
            for cp in wcopies((h + 1) // 2, ((h + 1) // 2) % 2):
                cp.wait()

        @pl.when(jnp.logical_and(h % 2 == 0, h + 2 < H))
        def _():
            for cp in wcopies(h // 2 + 1, (h // 2 + 1) % 2):
                cp.start()
        for i in range(4):
            @pl.when(h == 2 * i + 2)
            def _():
                for cp in big[i]:
                    cp.start()
        a, p = att_steps(h), proj_steps(h + 1)
        pos = 0
        for n, f in enumerate(a):
            f()
            for g in p[pos:PLACE[n]]:
                g()
            pos = PLACE[n]
        return 0
    lax.fori_loop(0, H - 1, body, 0)
    for f in att_steps(jnp.int32(H - 1)):
        f()

    for cp in big[0]:
        cp.wait()
    wr = wr_ref[...].astype(f32).reshape(1, M)
    sub = lax.broadcasted_iota(i32, (8, 1), 0)

    NG = M // T
    RG = RC // NG

    def mm(i, j):
        rows = pl.ds(pl.multiple_of(i * RC, RC), RC)
        a_v[i % 2, :, j * T:(j + 1) * T] = _dot(_cat([ctx_v[h, rows, :] for h in range(H)], 1), wo_v[j])

    def ocopy(i):
        rows = pl.ds(pl.multiple_of(i * RC, RC), RC)
        return pltpu.make_async_copy(out_v.at[rows, :], out_hbm.at[rows, :], osems.at[i])

    def epi(i, j, carry):
        m1, i1, m2, i2 = carry
        rows = pl.ds(pl.multiple_of(i * RC + j * RG, RG), RG)
        h = _rb(x_v[rows, :].astype(f32) + _rb(a_v[i % 2, j * RG:(j + 1) * RG, :]))
        m = jnp.mean(h, axis=-1, keepdims=True)
        hc = h - m
        v = jnp.mean(hc * hc, axis=-1, keepdims=True)
        d = _rb(jnp.sqrt(_rb(_rb(v) + EPS)))
        inv = pl.reciprocal(d, approx=True)
        inv = inv * (2.0 - d * inv)
        inv = inv * (2.0 - d * inv)
        hn = (_rb(h - _rb(m)) * inv).astype(bf16)
        x_v[rows, :] = h.astype(bf16)
        for c in range(M // T):
            xn_v[c, rows, :] = hn[:, c * T:(c + 1) * T]
        hn = hn.astype(f32)
        out_v[rows, :] = (h + hn).astype(bf16)
        r = _rb(jnp.sum(hn * wr, axis=1, keepdims=True))
        for g in range(RG // 8):
            v = r[g * 8:(g + 1) * 8]
            idx = sub + (i * RC + j * RG + g * 8)
            g1, g2 = v > m1, v > m2
            m2, i2 = jnp.where(g1, m1, jnp.where(g2, v, m2)), jnp.where(g1, i1, jnp.where(g2, idx, i2))
            m1, i1 = jnp.where(g1, v, m1), jnp.where(g1, idx, i1)
        return m1, i1, m2, i2

    ninf = jnp.full((8, 1), -jnp.inf, f32)
    zero = jnp.zeros((8, 1), i32)
    for j in range(NG):
        mm(jnp.int32(0), j)

    def obody(i, carry):
        for j in range(NG):
            carry = epi(i, j, carry)
            mm(i + 1, j)
        ocopy(i).start()
        return carry
    carry = lax.fori_loop(0, S // RC - 1, obody, (ninf, zero, ninf, zero))
    for j in range(NG):
        carry = epi(jnp.int32(S // RC - 1), j, carry)
    ocopy(jnp.int32(S // RC - 1)).start()
    m1, i1, m2, i2 = carry

    big_i = jnp.int32(S)
    va = jnp.max(m1)
    ia = jnp.min(jnp.where(m1 == va, i1, big_i))
    hit = i1 == ia
    n1, j1 = jnp.where(hit, m2, m1), jnp.where(hit, i2, i1)
    vb = jnp.max(n1)
    ib = jnp.min(jnp.where(n1 == vb, j1, big_i))
    ia = jnp.clip(ia, 0, S - 1); ib = jnp.clip(ib, 0, S - 1)
    ta = pl.multiple_of((ia // 16) * 16, 16)
    tb = pl.multiple_of((ib // 16) * 16, 16)

    for cp in big[1] + big[2] + big[3]:
        cp.wait()
    hn_tile = lambda t: _cat([xn_v[j, pl.ds(t, 16), :] for j in range(M // T)], 1)
    xs = _cat([hn_tile(ta), hn_tile(tb)], 0)
    wcat = lambda w: _cat([w[j] for j in range(w.shape[0])], 1)
    g = _rb(_dot(xs, wcat(wg_v)))
    u = _rb(_dot(xs, wcat(wu_v)))
    act = (_rb(g * jax.nn.sigmoid(g)) * u).astype(bf16)
    y = _rb(_dot(act, wcat(wd_v)))
    for i in range(S // RC):
        ocopy(i).wait()
    r16 = lax.broadcasted_iota(i32, (16, 1), 0)
    for k, (ii, tt, vv) in enumerate(((ia, ta, va), (ib, tb, vb))):
        yk = _rb(y[k * 16:(k + 1) * 16] * _rb(jax.nn.sigmoid(jnp.full((16, 1), vv, f32))))
        hn = hn_tile(tt).astype(f32)
        h = x_v[pl.ds(tt, 16), :].astype(f32)
        new = (h + _rb(hn + yk)).astype(bf16)
        out_v[pl.ds(tt, 16), :] = jnp.where(r16 + tt == ii, new, out_v[pl.ds(tt, 16), :])
    fin = [pltpu.make_async_copy(out_v.at[pl.ds(tt, 16), :], out_hbm.at[pl.ds(tt, 16), :], osems.at[k])
           for k, tt in enumerate((ta, tb))]
    fin[0].start()

    @pl.when(ta != tb)
    def _():
        fin[1].start()
        fin[1].wait()
    fin[0].wait()


@jax.jit
def pallas_sequential_preLN__compressed_kv_cla__moe_arch_mod__prompt_kernel(
        A_x, A_c_kv, A_w_q, A_w_uk, A_w_uv, A_w_o, B_x, B_w_r, B_w_gate, B_w_up, B_w_down):
    del B_x
    any_ = pl.BlockSpec(memory_space=pl.ANY)
    vm = pltpu.VMEM
    out = pl.pallas_call(
        _kernel,
        in_specs=[any_] * 6 + [pl.BlockSpec(memory_space=vm)] + [any_] * 3,
        out_specs=any_,
        out_shape=jax.ShapeDtypeStruct((S, M), bf16),
        scratch_shapes=[
            vm((S, M), bf16), vm((M // T, S, T), bf16), vm((DC // T, S, T), bf16),
            vm((2, M, D), u32), vm((2, DC, D), u32), vm((2, DC, D), u32),
            vm((2, S, D), bf16), vm((2, S, D), bf16), vm((2, S, D), bf16),
            vm((H, S, D), bf16), vm((M // T, H * D, T), bf16),
            vm((F // T, M, T), bf16), vm((F // T, M, T), bf16), vm((M // T, F, T), bf16),
            vm((S, M), bf16), vm((2, RC, M), f32),
            pltpu.SemaphoreType.DMA((12,)), pltpu.SemaphoreType.DMA((DC // T,)), pltpu.SemaphoreType.DMA((S // RC,)),
        ],
        compiler_params=pltpu.CompilerParams(vmem_limit_bytes=112 * 2**20),
    )(A_x.reshape(S, M), A_c_kv.reshape(S, DC), A_w_q, A_w_uk, A_w_uv, A_w_o.reshape(H * D, M),
      B_w_r, B_w_gate, B_w_up, B_w_down)
    return out.reshape(1, S, M)
```

```python
import functools
import jax, jax.numpy as jnp
from jax import lax
from jax.experimental import pallas as pl
from jax.experimental.pallas import tpu as pltpu

S, M, H, D, DC, F = 2048, 1024, 32, 128, 512, 3584
BQ = 512
T = 128
RC = 256
XC = 256
AHEAD = 2
LG = 16
PC = 512
LOOK = 1
PLACE = (3,3,6,6,9,9,12,15)
f32, bf16, u32, i32 = jnp.float32, jnp.bfloat16, jnp.uint32, jnp.int32
QSC = (D ** -0.5) * 1.4426950408889634
NEG = -1e30
EPS = 1e-5


def _dot(a, b):
    return jnp.dot(a, b, preferred_element_type=f32)


def _dot_nt(a, b):
    return lax.dot_general(a, b, (((1,), (1,)), ((), ())), preferred_element_type=f32)


def _rb(x):
    return x.astype(bf16).astype(f32)


def _cat(xs, axis):
    return xs[0] if len(xs) == 1 else jnp.concatenate(xs, axis=axis)


def _tiles(x):
    return [x[:, j * T:(j + 1) * T] for j in range(x.shape[1] // T)]


def _attend_steps(q_ref, k_ref, v_ref, o_ref, bias):
    nt = BQ // T

    def qk(I):
        r0 = I * BQ
        q = q_ref[r0:r0 + BQ, :]
        sr = _tiles(_dot_nt(q, k_ref[:r0, :])) if I else []
        sd = [_dot_nt(q[t * T:], k_ref[r0 + t * T:r0 + (t + 1) * T, :]) for t in range(nt)]
        return sr, sd

    def softmax(s):
        sr, sd = s
        n = len(sr)
        pd = [[] for _ in range(nt)]
        pr, ls = [], []
        for r in range(nt):
            pcs = [x[r * T:(r + 1) * T] for x in sr] + [sd[t][(r - t) * T:(r - t + 1) * T] for t in range(r + 1)]
            pcs[-1] = pcs[-1] + bias
            m = jnp.max(functools.reduce(jnp.maximum, pcs), axis=1, keepdims=True)
            ps = [jnp.exp2(x - m).astype(bf16) for x in pcs]
            ls.append(jnp.sum(functools.reduce(jnp.add, [x.astype(f32) for x in ps]), axis=1, keepdims=True))
            if n:
                pr.append(_cat(ps[:n], 1))
            for t in range(r + 1):
                pd[t].append(ps[n + t])
        return pr, pd, ls

    def pv(I, p):
        pr, pd, ls = p
        r0 = I * BQ
        orr = _dot(_cat(pr, 0), v_ref[:r0, :]) if I else None
        os_ = [_dot(_cat(pd[t], 0), v_ref[r0 + t * T:r0 + (t + 1) * T, :]) for t in range(nt)]
        for r in range(nt):
            pcs = [os_[t][(r - t) * T:(r - t + 1) * T] for t in range(r + 1)]
            if I:
                pcs.append(orr[r * T:(r + 1) * T])
            l = ls[r]
            inv = pl.reciprocal(l, approx=True)
            inv = inv * (2.0 - l * inv)
            o_ref[r0 + r * T:r0 + (r + 1) * T, :] = (functools.reduce(jnp.add, pcs) * inv).astype(bf16)

    order = list(range(S // BQ))[::-1]
    st = {}
    QK = [lambda n=n: st.__setitem__(n, qk(order[n])) for n in range(len(order))]
    SP = [lambda n=n: pv(order[n], softmax(st.pop(n))) for n in range(len(order))]
    steps = QK[:LOOK]
    for n in range(len(order)):
        if n + LOOK < len(order):
            steps.append(QK[n + LOOK])
        steps.append(SP[n])
    return steps


def _kernel(x_hbm, c_hbm, wq_hbm, wk_hbm, wv_hbm, wo_hbm, wr_ref, wg_hbm, wu_hbm, wd_hbm, out_hbm,
            x_v, xn_v, c_v, wq_r, wk_r, wv_r, q_v, k_v, v_v, ctx_v, wo_v, wg_v, wu_v, wd_v, out_v, a_v,
            sems, csems, osems):
    wq32, wk32, wv32 = wq_hbm.bitcast(u32), wk_hbm.bitcast(u32), wv_hbm.bitcast(u32)

    def wcopies(p, s):
        return (pltpu.make_async_copy(wq32.at[:, p, :], wq_r.at[s], sems.at[s]),
                pltpu.make_async_copy(wk32.at[:, p, :], wk_r.at[s], sems.at[2 + s]),
                pltpu.make_async_copy(wv32.at[:, p, :], wv_r.at[s], sems.at[4 + s]))
    NX = S // XC
    cp_c = [[pltpu.make_async_copy(c_hbm.at[i * XC:(i + 1) * XC, j * T:(j + 1) * T], c_v.at[j, i * XC:(i + 1) * XC], csems.at[i])
             for j in range(DC // T)] for i in range(NX)]
    cp_x = [pltpu.make_async_copy(x_hbm.at[i * XC:(i + 1) * XC], x_v.at[i * XC:(i + 1) * XC], osems.at[i]) for i in range(NX)]

    def tile_copy(i, src, dst, j, r0=0, n=None):
        n = n or dst.shape[1]
        return pltpu.make_async_copy(src.at[pl.ds(r0, n), pl.ds(j * T, T)], dst.at[j, pl.ds(r0, n), :], sems.at[8 + i])

    def big_start(j):
        for e in range(2):
            tile_copy(1, wg_hbm, wg_v, 2 * j + e).start()
            tile_copy(2, wu_hbm, wu_v, 2 * j + e).start()

    def big_start2(j):
        tile_copy(0, wo_hbm, wo_v, j // 2, (j % 2) * (H * D // 2), H * D // 2).start()
        tile_copy(3, wd_hbm, wd_v, j // 2, (j % 2) * (F // 2), F // 2).start()

    def big_wait(i, dst):
        pltpu.make_async_copy(dst, dst, sems.at[8 + i]).wait()

    cq, ck, cv = wcopies(0, 0)
    ck.start(); cv.start(); cq.start()

    def chunk_start(i):
        for cp in cp_c[i]:
            cp.start()
        cp_x[i].start()
    for i in range(AHEAD):
        chunk_start(i)

    def unpack(ref, slot, a):
        w = ref[slot]
        w = (w << 16) if a == 0 else (w & jnp.uint32(0xFFFF0000))
        return pltpu.bitcast(w, f32).astype(bf16)

    def project(src, n, w, dst, sc, rows):
        r = _dot(_cat([src[j, rows, :] for j in range(n)], 1), w)
        dst[rows, :] = (r if sc is None else r * sc).astype(bf16)

    def proj_steps(slot, a):
        w = {}
        steps = []
        for name, raw, src, n, dst, sc in (("k", wk_r, c_v, DC // T, k_v, None), ("v", wv_r, c_v, DC // T, v_v, None),
                                           ("q", wq_r, xn_v, M // T, q_v, QSC)):
            steps.append(lambda name=name, raw=raw: w.__setitem__(name, unpack(raw, slot, a)))
            for i in range(S // PC):
                steps.append(lambda name=name, src=src, n=n, dst=dst, sc=sc, i=i: project(
                    src, n, w[name], dst.at[a], sc, slice(i * PC, (i + 1) * PC)))
        return steps

    ck.wait(); cv.wait()
    wk0, wv0 = unpack(wk_r, 0, 0), unpack(wv_r, 0, 0)
    cq.wait()
    wq0 = unpack(wq_r, 0, 0)
    for i in range(NX):
        rows = slice(i * XC, (i + 1) * XC)
        for cp in cp_c[i]:
            cp.wait()
        cp_x[i].wait()
        if i + AHEAD < NX:
            chunk_start(i + AHEAD)
        elif i + AHEAD == NX:
            for cp in wcopies(1, 1):
                cp.start()
        project(c_v, DC // T, wk0, k_v.at[0], None, rows)
        for g in range(XC // LG):
            rg = slice(i * XC + g * LG, i * XC + (g + 1) * LG)
            x = x_v[rg, :].astype(f32)
            xc = x - jnp.mean(x, axis=-1, keepdims=True)
            xn = (xc * lax.rsqrt(jnp.mean(xc * xc, axis=-1, keepdims=True) + EPS)).astype(bf16)
            for j in range(M // T):
                xn_v[j, rg, :] = xn[:, j * T:(j + 1) * T]
            if g == XC // LG // 2:
                project(c_v, DC // T, wv0, v_v.at[0], None, rows)
        if i:
            project(xn_v, M // T, wq0, q_v.at[0], QSC, slice((i - 1) * XC, i * XC))
    project(xn_v, M // T, wq0, q_v.at[0], QSC, slice(S - XC, S))

    row = lax.broadcasted_iota(i32, (T, T), 0)
    col = lax.broadcasted_iota(i32, (T, T), 1)
    bias = jnp.where(col <= row, 0.0, NEG).astype(f32)

    def head(h, a, nxt):
        st = _attend_steps(q_v.at[a], k_v.at[a], v_v.at[a], ctx_v.at[h], bias)
        p = proj_steps(*nxt) if nxt else []
        pos = 0
        for n, f in enumerate(st):
            f()
            for g in p[pos:PLACE[n]]:
                g()
            pos = PLACE[n]

    big_start2(15)
    head(0, 0, (0, 1))

    def body(j, _):
        s1 = (j + 1) % 2
        for cp in wcopies(j + 1, s1):
            cp.wait()

        @pl.when(j < 14)
        def _():
            for cp in wcopies(j + 2, j % 2):
                cp.start()
            big_start(j)
        big_start2(j)
        head(2 * j + 1, 1, (s1, 0))
        head(2 * j + 2, 0, (s1, 1))
        return 0
    lax.fori_loop(0, H // 2 - 1, body, 0)
    head(H - 1, 1, None)

    big_wait(0, wo_v)
    wr = wr_ref[...].astype(f32).reshape(1, M)
    sub = lax.broadcasted_iota(i32, (8, 1), 0)

    NG = M // T
    RG = RC // NG

    def mm(i, j):
        rows = pl.ds(pl.multiple_of(i * RC, RC), RC)
        a_v[i % 2, :, j * T:(j + 1) * T] = _dot(_cat([ctx_v[h, rows, :] for h in range(H)], 1), wo_v[j])

    def ocopy(i):
        rows = pl.ds(pl.multiple_of(i * RC, RC), RC)
        return pltpu.make_async_copy(out_v.at[rows, :], out_hbm.at[rows, :], osems.at[i])

    def epi(i, j, carry):
        m1, i1, m2, i2 = carry
        rows = pl.ds(pl.multiple_of(i * RC + j * RG, RG), RG)
        h = _rb(x_v[rows, :].astype(f32) + _rb(a_v[i % 2, j * RG:(j + 1) * RG, :]))
        m = jnp.mean(h, axis=-1, keepdims=True)
        hc = h - m
        v = jnp.mean(hc * hc, axis=-1, keepdims=True)
        d = _rb(jnp.sqrt(_rb(_rb(v) + EPS)))
        inv = pl.reciprocal(d, approx=True)
        inv = inv * (2.0 - d * inv)
        inv = inv * (2.0 - d * inv)
        hn = (_rb(h - _rb(m)) * inv).astype(bf16)
        x_v[rows, :] = h.astype(bf16)
        for c in range(M // T):
            xn_v[c, rows, :] = hn[:, c * T:(c + 1) * T]
        hn = hn.astype(f32)
        out_v[rows, :] = (h + hn).astype(bf16)
        r = _rb(jnp.sum(hn * wr, axis=1, keepdims=True))
        for g in range(RG // 8):
            v = r[g * 8:(g + 1) * 8]
            idx = sub + (i * RC + j * RG + g * 8)
            g1, g2 = v > m1, v > m2
            m2, i2 = jnp.where(g1, m1, jnp.where(g2, v, m2)), jnp.where(g1, i1, jnp.where(g2, idx, i2))
            m1, i1 = jnp.where(g1, v, m1), jnp.where(g1, idx, i1)
        return m1, i1, m2, i2

    ninf = jnp.full((8, 1), -jnp.inf, f32)
    zero = jnp.zeros((8, 1), i32)
    for j in range(NG):
        mm(jnp.int32(0), j)

    def obody(i, carry):
        for j in range(NG):
            carry = epi(i, j, carry)
            mm(i + 1, j)
        ocopy(i).start()
        return carry
    carry = lax.fori_loop(0, S // RC - 1, obody, (ninf, zero, ninf, zero))
    for j in range(NG):
        carry = epi(jnp.int32(S // RC - 1), j, carry)
    ocopy(jnp.int32(S // RC - 1)).start()
    m1, i1, m2, i2 = carry

    big_i = jnp.int32(S)
    va = jnp.max(m1)
    ia = jnp.min(jnp.where(m1 == va, i1, big_i))
    hit = i1 == ia
    n1, j1 = jnp.where(hit, m2, m1), jnp.where(hit, i2, i1)
    vb = jnp.max(n1)
    ib = jnp.min(jnp.where(n1 == vb, j1, big_i))
    ia = jnp.clip(ia, 0, S - 1); ib = jnp.clip(ib, 0, S - 1)
    ta = pl.multiple_of((ia // 16) * 16, 16)
    tb = pl.multiple_of((ib // 16) * 16, 16)

    big_wait(1, wg_v); big_wait(2, wu_v); big_wait(3, wd_v)
    hn_tile = lambda t: _cat([xn_v[j, pl.ds(t, 16), :] for j in range(M // T)], 1)
    xs = _cat([hn_tile(ta), hn_tile(tb)], 0)
    wcat = lambda w: _cat([w[j] for j in range(w.shape[0])], 1)
    g = _rb(_dot(xs, wcat(wg_v)))
    u = _rb(_dot(xs, wcat(wu_v)))
    act = (_rb(g * jax.nn.sigmoid(g)) * u).astype(bf16)
    y = _rb(_dot(act, wcat(wd_v)))
    for i in range(S // RC):
        ocopy(i).wait()
    r16 = lax.broadcasted_iota(i32, (16, 1), 0)
    for k, (ii, tt, vv) in enumerate(((ia, ta, va), (ib, tb, vb))):
        yk = _rb(y[k * 16:(k + 1) * 16] * _rb(jax.nn.sigmoid(jnp.full((16, 1), vv, f32))))
        hn = hn_tile(tt).astype(f32)
        h = x_v[pl.ds(tt, 16), :].astype(f32)
        new = (h + _rb(hn + yk)).astype(bf16)
        out_v[pl.ds(tt, 16), :] = jnp.where(r16 + tt == ii, new, out_v[pl.ds(tt, 16), :])
    fin = [pltpu.make_async_copy(out_v.at[pl.ds(tt, 16), :], out_hbm.at[pl.ds(tt, 16), :], osems.at[k])
           for k, tt in enumerate((ta, tb))]
    fin[0].start()

    @pl.when(ta != tb)
    def _():
        fin[1].start()
        fin[1].wait()
    fin[0].wait()


@jax.jit
def pallas_sequential_preLN__compressed_kv_cla__moe_arch_mod__prompt_kernel(
        A_x, A_c_kv, A_w_q, A_w_uk, A_w_uv, A_w_o, B_x, B_w_r, B_w_gate, B_w_up, B_w_down):
    del B_x
    any_ = pl.BlockSpec(memory_space=pl.ANY)
    vm = pltpu.VMEM
    out = pl.pallas_call(
        _kernel,
        in_specs=[any_] * 6 + [pl.BlockSpec(memory_space=vm)] + [any_] * 3,
        out_specs=any_,
        out_shape=jax.ShapeDtypeStruct((S, M), bf16),
        scratch_shapes=[
            vm((S, M), bf16), vm((M // T, S, T), bf16), vm((DC // T, S, T), bf16),
            vm((2, M, D), u32), vm((2, DC, D), u32), vm((2, DC, D), u32),
            vm((2, S, D), bf16), vm((2, S, D), bf16), vm((2, S, D), bf16),
            vm((H, S, D), bf16), vm((M // T, H * D, T), bf16),
            vm((F // T, M, T), bf16), vm((F // T, M, T), bf16), vm((M // T, F, T), bf16),
            vm((S, M), bf16), vm((2, RC, M), f32),
            pltpu.SemaphoreType.DMA((12,)), pltpu.SemaphoreType.DMA((S // XC,)), pltpu.SemaphoreType.DMA((S // RC,)),
        ],
        compiler_params=pltpu.CompilerParams(vmem_limit_bytes=112 * 2**20),
    )(A_x.reshape(S, M), A_c_kv.reshape(S, DC), A_w_q, A_w_uk, A_w_uv, A_w_o.reshape(H * D, M),
      B_w_r, B_w_gate, B_w_up, B_w_down)
    return out.reshape(1, S, M)
```
